```python
import jax
import jax.numpy as jnp

def _softmax(x, axis=-1):
    return jax.nn.softmax(x, axis=axis)
def _gelu(x):
    return jax.nn.gelu(x, approximate=True)
def _silu(x):
    return jax.nn.silu(x)
def _sigmoid(x):
    return jax.nn.sigmoid(x)
def _layernorm(x, axis=-1, eps=1e-5):
    m = jnp.mean(x, axis=axis, keepdims=True)
    v = jnp.var(x, axis=axis, keepdims=True)
    return (x - m) / jnp.sqrt(v + eps)
def _scatter_add(tgt, idx, src, axis=0):
    return tgt.at[idx].add(src)
def _segment_sum(src, seg, n):
    return jax.ops.segment_sum(src, seg, n)
class _Rng:
    def __init__(self, key):
        self._k = key
    def _next(self):
        self._k, sub = jax.random.split(self._k)
        return sub
    def normal(self, shape):
        return jax.random.normal(self._next(), shape, dtype=jnp.bfloat16)
    def randint(self, lo, hi, shape):
        return jax.random.randint(self._next(), shape, lo, hi, dtype=jnp.int32)
    def uniform(self, shape, lo=0.0, hi=1.0):
        return jax.random.uniform(self._next(), shape, jnp.bfloat16, lo, hi)
    def permutation(self, n):
        return jax.random.permutation(self._next(), n)


kernel_name = 'standalone__batchnorm__prompt'

def setup_inputs():
    _rng = _Rng(jax.random.key(int.from_bytes(__import__("os").urandom(4), "little")))
    _w = (lambda a: (lambda t: t.astype(jnp.bfloat16) if jnp.issubdtype(t.dtype, jnp.floating) else t)(jnp.asarray(a)))
    B, S, C = 2, 2048, 1024
    K = 3
    return {
        "x": _w((lambda *s: _rng.normal(s) * 0.05)(B, S, C)),
        "w": _w((lambda *s: _rng.normal(s) * 0.05)(K, C, C) * (1.0 / (K * C) ** 0.5)),
        "mean": _w((lambda *s: _rng.normal(s) * 0.05)(C) * 0.1),
        "var": _w(jnp.abs((lambda *s: _rng.normal(s) * 0.05)(C)) + 0.5),
        "g": _w((lambda *s: _rng.normal(s) * 0.05)(C) + 1.0),
        "b": _w((lambda *s: _rng.normal(s) * 0.05)(C) * 0.1),
    }

def reference(x, w, mean, var, g, b):
    K = 3
    P = K // 2
    S = x.shape[1]
    xp = jnp.pad(x, ((0, 0), (P, P), (0, 0)))
    y = sum(jnp.einsum('bsc,cd->bsd', xp[:, k:k + S, :], w[k]) for k in range(K))
    inv_std = 1.0 / jnp.sqrt(var + 1e-5)
    y = (y - mean) * (g * inv_std) + b
    return _silu(y)
```

```python
import jax
import jax.numpy as jnp
from jax.experimental import pallas as pl
from jax.experimental.pallas import tpu as pltpu


TM = 256
TN = 128
H = 16
AHEAD = 2


def _make_kernel(B, S, C, K):
    nt = S // TM
    T = B * nt
    NN = C // TN
    bf, f32 = jnp.bfloat16, jnp.float32
    h = TM // 2
    r = lambda a: a.astype(bf).astype(f32)

    def kern(x_hbm, w_hbm, mean_ref, var_ref, g_ref, b_ref, o_hbm,
             xs, ws, wsu, lhs, ob, yb, pv, xsem, wsem, osem):
        def x_rows(t):
            i = t % nt
            lo = 0 if i == 0 else i * TM + H
            return lo, min(S, (i + 1) * TM + H)

        def xcopy(t):
            lo, hi = x_rows(t)
            return pltpu.make_async_copy(
                x_hbm.at[t // nt, pl.ds(lo, hi - lo)],
                xs.at[t // nt, pl.ds(H + lo, hi - lo)], xsem.at[t])

        def wcopy(n):
            return pltpu.make_async_copy(
                w_hbm.at[:, pl.ds(n * TN, TN)], ws.at[:, pl.ds(n * TN, TN)],
                wsem.at[n])

        def ocopy(t, slot):
            i = t % nt
            r0 = i * TM if isinstance(t, int) else pl.multiple_of(i * TM, TM)
            return pltpu.make_async_copy(
                ob.at[slot], o_hbm.at[t // nt, pl.ds(r0, TM)], osem.at[slot])

        queue = ([xcopy(0)] + [wcopy(n) for n in range(NN)]
                 + [xcopy(t) for t in range(1, T)])
        started = [0]

        def issue(upto):
            while started[0] < min(upto, len(queue)):
                queue[started[0]].start()
                started[0] += 1

        issue(1 + AHEAD)

        zeros = jnp.zeros((H, C), bf)
        for bb in range(B):
            xs[bb, 0:H] = zeros
            xs[bb, H + S:H + S + H] = zeros

        ld = lambda ref: ref[...].reshape(1, C).astype(f32)
        inv_std = r(1.0 / r(jnp.sqrt(r(ld(var_ref) + 1e-5))))
        pv[0:1] = r(ld(g_ref) * inv_std)
        pv[1:2] = ld(mean_ref)
        pv[2:3] = ld(b_ref)

        def epilogue(slot, n):
            cs = slice(n * TN, (n + 1) * TN)
            y = yb[n % 2].astype(f32)
            y = r(r(r(y - pv[1:2, cs]) * pv[0:1, cs]) + pv[2:3, cs])
            d = r(1.0 + r(jnp.exp(-y)))
            sg = r(pl.reciprocal(d, approx=True))
            ob[slot, :, cs] = (y * sg).astype(bf)

        def xwait_dyn(t):
            i = t % nt

            def wait_rows(n_rows):
                pltpu.make_async_copy(
                    x_hbm.at[0, pl.ds(0, n_rows)], xs.at[0, pl.ds(0, n_rows)],
                    xsem.at[t]).wait()

            @pl.when(i == 0)
            def _():
                @pl.when(t < T)
                def _():
                    wait_rows(TM + H)

            @pl.when(i == nt - 1)
            def _():
                wait_rows(TM - H)

            @pl.when((i > 0) & (i < nt - 1))
            def _():
                wait_rows(TM)

        def build(t, n):
            sl = t % 2
            if isinstance(t, int):
                r0 = (t % nt) * TM
            else:
                t = jnp.minimum(t, T - 1)
                r0 = pl.multiple_of((t % nt) * TM, TM)
            c0, c1 = n * TN, (n + 1) * TN
            u = pltpu.bitcast(xs[t // nt, pl.ds(r0, TM + 2 * H), c0:c1],
                              jnp.uint32)
            up, uc, un = u[7:7 + h], u[8:8 + h], u[9:9 + h]
            lhs[sl, :, c0:c1] = (up >> 16) | (uc << 16)
            lhs[sl, :, C + c0:C + c1] = uc
            lhs[sl, :, 2 * C + c0:2 * C + c1] = (uc >> 16) | (un << 16)

        def tile(t, first):
            slot = t % 2
            if first:
                xcopy(0).wait()
                for n in range(NN):
                    build(0, n)
            else:
                xwait_dyn(t + 1)

                @pl.when(t >= 2)
                def _():
                    ocopy(t - 2, slot).wait()

            for n in range(NN):
                cs = slice(n * TN, (n + 1) * TN)
                if first:
                    wcopy(n).wait()
                    issue(n + 2 + AHEAD)
                    wsu[:, cs] = pltpu.bitcast(ws[:, cs], jnp.uint32)
                for k in range(K):
                    a_ = pltpu.bitcast(lhs[slot, :, k * C:(k + 1) * C], bf)
                    b_ = pltpu.bitcast(
                        wsu[k * C // 2:(k + 1) * C // 2, cs], bf)
                    p = r(jnp.dot(a_, b_, preferred_element_type=f32))
                    y = p if k == 0 else (
                        r(y + p) if k < K - 1 else (y + p).astype(bf))
                yb[n % 2] = y
                if n > 0:
                    epilogue(slot, n - 1)
                elif not first:
                    epilogue(1 - slot, NN - 1)
                if first:
                    if n == NN - 1:
                        issue(NN + 2)
                        xcopy(1).wait()
                        for n2 in range(NN):
                            build(1, n2)
                else:
                    build(t + 1, n)
                if n == 0 and not first:
                    ocopy(t - 1, 1 - slot).start()
            if first:
                issue(len(queue))

        tile(0, True)

        def body(t, c):
            tile(t, False)
            return c

        jax.lax.fori_loop(1, T, body, 0)
        epilogue((T - 1) % 2, NN - 1)
        ocopy(T - 1, (T - 1) % 2).start()
        ocopy(T - 2, T % 2).wait()
        ocopy(T - 1, (T - 1) % 2).wait()

    return kern, T, NN


@jax.jit
def pallas_standalone__batchnorm__prompt_kernel(
    x: jax.Array,
    w: jax.Array,
    mean: jax.Array,
    var: jax.Array,
    g: jax.Array,
    b: jax.Array,
):
    B, S, C = x.shape
    K = w.shape[0]
    bf = jnp.bfloat16
    kern, T, NN = _make_kernel(B, S, C, K)
    hbm = pl.BlockSpec(memory_space=pltpu.HBM)
    vmem = pl.BlockSpec(memory_space=pltpu.VMEM)
    return pl.pallas_call(
        kern,
        in_specs=[hbm, hbm, vmem, vmem, vmem, vmem],
        out_specs=hbm,
        out_shape=jax.ShapeDtypeStruct((B, S, C), bf),
        scratch_shapes=[
            pltpu.VMEM((B, S + 2 * H, C), bf),
            pltpu.VMEM((K * C, C), bf),
            pltpu.VMEM((K * C // 2, C), jnp.uint32),
            pltpu.VMEM((2, TM // 2, K * C), jnp.uint32),
            pltpu.VMEM((2, TM, C), bf),
            pltpu.VMEM((2, TM, TN), bf),
            pltpu.VMEM((8, C), jnp.float32),
            pltpu.SemaphoreType.DMA((T,)),
            pltpu.SemaphoreType.DMA((NN,)),
            pltpu.SemaphoreType.DMA((2,)),
        ],
        compiler_params=pltpu.CompilerParams(vmem_limit_bytes=64 * 2**20),
    )(x, w.reshape(K * C, C), mean, var, g, b)
```

```python
import jax
import jax.numpy as jnp
from jax.experimental import pallas as pl
from jax.experimental.pallas import tpu as pltpu

TM = 512
T1 = 256
TN = 128
H = 16
AHEAD = 3
NPC = 8
W_GROUPS = ((0,), (1,), (2, 3), (4, 5), (6, 7))


def _make_kernel(B, S, C, K):
    nt = S // TM
    T = B * nt
    NN = C // TN
    P = TM // T1
    bf, f32, u32 = jnp.bfloat16, jnp.float32, jnp.uint32
    r = lambda a: a.astype(bf).astype(f32)

    xch = [(0, 0 if c == 0 else c * T1 + H, (c + 1) * T1 + H) for c in range(P)]
    for t in range(1, T):
        i = t % nt
        xch.append((t // nt, 0 if i == 0 else i * TM + H,
                    min(S, (i + 1) * TM + H)))

    names = ([("x", 0), ("w", 0)] + [("x", c) for c in range(1, P)]
             + [("w", n) for n in range(1, 4)] + [("x", P)]
             + [("w", n) for n in range(4, NN)]
             + [("x", c) for c in range(P + 1, len(xch))])
    pos = {nm: j for j, nm in enumerate(names)}

    def kern(x_hbm, w_hbm, mean_hbm, var_hbm, g_hbm, b_hbm, o_hbm,
             xs, wsu, lhs, ob, yb, pv, pb0, pb1, pb2, pb3,
             xsem, wsem, osem, psem):
        pvb = (pb0, pb1, pb2, pb3)
        pcopies = [
            pltpu.make_async_copy(src, pvb[j], psem.at[j])
            for j, src in enumerate((mean_hbm, var_hbm, g_hbm, b_hbm))
        ]

        def params():
            for c in pcopies:
                c.wait()
            ld = lambda j: pvb[j][...].reshape(1, C).astype(f32)
            inv_std = r(1.0 / r(jnp.sqrt(r(ld(1) + 1e-5))))
            pv[0:1] = r(ld(2) * inv_std)
            pv[1:2] = ld(0)
            pv[2:3] = ld(3)

        def xcopy(c):
            bb, lo, hi = xch[c]
            return pltpu.make_async_copy(
                x_hbm.at[bb, pl.ds(lo, hi - lo)],
                xs.at[bb, pl.ds(H + lo, hi - lo)], xsem.at[c])

        def wcopy(n):
            cs = pl.ds(n * TN, TN)
            return pltpu.make_async_copy(
                w_hbm.bitcast(u32).at[:, cs], wsu.at[:, cs], wsem.at[n])

        def ocopy(t, c0=0, c1=C):
            i = t % nt
            r0 = i * TM if isinstance(t, int) else pl.multiple_of(i * TM, TM)
            cs = pl.ds(c0, c1 - c0)
            return pltpu.make_async_copy(
                ob.at[t, :, cs], o_hbm.at[t // nt, pl.ds(r0, TM), cs],
                osem.at[0])

        queue = [xcopy(i) if kind == "x" else wcopy(i) for kind, i in names]
        started = [0]

        def issue(upto):
            while started[0] < min(upto, len(queue)):
                queue[started[0]].start()
                started[0] += 1

        def need(nm):
            issue(pos[nm] + 1)
            queue[pos[nm]].wait()
            issue(pos[nm] + 1 + AHEAD)

        def xwait_dyn(t):
            i = t % nt

            def wait_rows(n_rows):
                pltpu.make_async_copy(
                    x_hbm.at[0, pl.ds(0, n_rows)], xs.at[0, pl.ds(0, n_rows)],
                    xsem.at[P - 1 + t]).wait()

            @pl.when(i == 0)
            def _():
                @pl.when(t < T)
                def _():
                    wait_rows(TM + H)

            @pl.when(i == nt - 1)
            def _():
                wait_rows(TM - H)

            @pl.when((i > 0) & (i < nt - 1))
            def _():
                wait_rows(TM)

        def build(bb, s0, slot, q0, nr, n):
            h = nr // 2
            c0, c1 = n * TN, (n + 1) * TN
            u = pltpu.bitcast(xs[bb, pl.ds(s0, nr + 2 * H), c0:c1], u32)
            lo = H // 2
            up, uc, un = u[lo - 1:lo - 1 + h], u[lo:lo + h], u[lo + 1:lo + 1 + h]
            lhs[slot, q0:q0 + h, c0:c1] = (up >> 16) | (uc << 16)
            lhs[slot, q0:q0 + h, C + c0:C + c1] = uc
            lhs[slot, q0:q0 + h, 2 * C + c0:2 * C + c1] = (uc >> 16) | (un << 16)

        def build_tile(t, n):
            if isinstance(t, int):
                build(t // nt, (t % nt) * TM, t % 2, 0, TM, n)
            else:
                tt = jnp.minimum(t, T - 1)
                build(tt // nt, pl.multiple_of((tt % nt) * TM, TM), t % 2, 0,
                      TM, n)

        def dots(t, y0, nr, n):
            cs = slice(n * TN, (n + 1) * TN)
            h, q0 = nr // 2, y0 // 2
            for k in range(K):
                a_ = pltpu.bitcast(lhs[t % 2, q0:q0 + h, k * C:(k + 1) * C], bf)
                b_ = pltpu.bitcast(wsu[k * C // 2:(k + 1) * C // 2, cs], bf)
                p = r(jnp.dot(a_, b_, preferred_element_type=f32))
                if k == 0:
                    y = p
                elif k < K - 1:
                    y = r(y + p)
                else:
                    y = (y + p).astype(bf)
            yb[n % 2, y0:y0 + nr] = y

        def epilogue(t, n, lo, hi, npieces, chain):
            cs = slice(n * TN, (n + 1) * TN)
            rp = (hi - lo) // npieces
            for i in range(npieces):
                a, b_ = lo + i * rp, lo + (i + 1) * rp
                y = yb[n % 2, a:b_].astype(f32)
                if chain is not None and chain.get("prev") is not None:
                    never = jnp.broadcast_to(pv[3:4, 0:TN], y.shape) != 0
                    y = jnp.where(never, chain["prev"], y)
                y = r(r(r(y - pv[1:2, cs]) * pv[0:1, cs]) + pv[2:3, cs])
                d = r(1.0 + r(jnp.exp(-y)))
                sg = r(pl.reciprocal(d, approx=True))
                o = y * sg
                ob[t, a:b_, cs] = o.astype(bf)
                if chain is not None:
                    chain["prev"] = o

        issue(2)
        for c in pcopies:
            c.start()
        zeros = jnp.zeros((H, C), bf)
        pv[3:4] = jnp.zeros((1, C), f32)
        for bb in range(B):
            xs[bb, 0:H] = zeros
            xs[bb, H + S:H + S + H] = zeros
        need(("x", 0))
        for n in range(NN):
            build(0, 0, 0, 0, T1, n)

        units = [(c, n) for n in range(NN) for c in range(P)]
        nu = len(units)
        for j, (c, n) in enumerate(units):
            if c == 0:
                for grp in W_GROUPS:
                    if grp[0] == n:
                        for n_ in grp:
                            need(("w", n_))
            if n == 0 and c > 0:
                need(("x", c))
                for n2 in range(NN):
                    build(0, c * T1, 0, c * T1 // 2, T1, n2)
            dots(0, c * T1, T1, n)
            if j == P:
                params()
            if n > 0:
                epilogue(0, n - 1, c * T1, (c + 1) * T1, 4, None)
            if j == nu - NN:
                need(("x", P))
            if j >= nu - NN:
                build_tile(1, j - (nu - NN))
        issue(len(queue))

        def body(t, carry):
            xwait_dyn(t + 1)
            chain = {}
            for n in range(NN):
                dots(t, 0, TM, n)
                if n > 0:
                    epilogue(t, n - 1, 0, TM, NPC, chain)
                else:
                    epilogue(t - 1, NN - 1, 0, TM, NPC, chain)
                    ocopy(t - 1).start()
                build_tile(t + 1, n)
            return carry

        jax.lax.fori_loop(1, T, body, 0)

        ocopy(T - 1, 0, C - TN).start()
        epilogue(T - 1, NN - 1, 0, TM, 1, None)
        ocopy(T - 1, C - TN, C).start()
        for t in range(T - 1):
            ocopy(t).wait()
        ocopy(T - 1, 0, C - TN).wait()
        ocopy(T - 1, C - TN, C).wait()

    return kern, T, NN, P


@jax.jit
def pallas_standalone__batchnorm__prompt_kernel(
    x: jax.Array,
    w: jax.Array,
    mean: jax.Array,
    var: jax.Array,
    g: jax.Array,
    b: jax.Array,
):
    B, S, C = x.shape
    K = w.shape[0]
    bf = jnp.bfloat16
    kern, T, NN, P = _make_kernel(B, S, C, K)
    hbm = pl.BlockSpec(memory_space=pltpu.HBM)
    return pl.pallas_call(
        kern,
        in_specs=[hbm] * 6,
        out_specs=hbm,
        out_shape=jax.ShapeDtypeStruct((B, S, C), bf),
        scratch_shapes=[
            pltpu.VMEM((B, S + 2 * H, C), bf),
            pltpu.VMEM((K * C // 2, C), jnp.uint32),
            pltpu.VMEM((2, TM // 2, K * C), jnp.uint32),
            pltpu.VMEM((T, TM, C), bf),
            pltpu.VMEM((2, TM, TN), bf),
            pltpu.VMEM((8, C), jnp.float32),
            pltpu.VMEM((C,), bf), pltpu.VMEM((C,), bf),
            pltpu.VMEM((C,), bf), pltpu.VMEM((C,), bf),
            pltpu.SemaphoreType.DMA((P - 1 + T,)),
            pltpu.SemaphoreType.DMA((NN,)),
            pltpu.SemaphoreType.DMA((1,)),
            pltpu.SemaphoreType.DMA((4,)),
        ],
        compiler_params=pltpu.CompilerParams(vmem_limit_bytes=80 * 2**20),
    )(x, w.reshape(K * C, C), mean, var, g, b)
```

```python
import jax
import jax.numpy as jnp
from jax.experimental import pallas as pl
from jax.experimental.pallas import tpu as pltpu

TM = 512
T1 = 256
TN = 128
H = 16
NPC = 8
OSPLIT = (4, 7, 8)
BUILD1 = (8, 14)
REST_AT = 2


def _make_kernel(B, S, C, K):
    nt = S // TM
    T = B * nt
    NN = C // TN
    P = TM // T1
    bf, f32, u32 = jnp.bfloat16, jnp.float32, jnp.uint32
    r = lambda a: a.astype(bf).astype(f32)

    xch = [(0, 0 if c == 0 else c * T1 + H, (c + 1) * T1 + H) for c in range(P)]
    for t in range(1, T):
        i = t % nt
        xch.append((t // nt, 0 if i == 0 else i * TM + H,
                    min(S, (i + 1) * TM + H)))

    groups = [
        ("pro", [("x", 0)]),
        (("k", 0), [("k", 0)]),
        (("k", 1), [("k", 1)]),
        (("k", 2), [("k", 2)]),
        (1, [("x", 1)]),
        (2, [("w", 1)]),
        (4, [("w", 2), ("w", 3)]),
        (8, [("x", 2), ("w", 4), ("w", 5)]),
        (12, [("w", 6), ("w", 7), ("x", 3)]),
        ("rest", [("x", c) for c in range(4, len(xch))]),
    ]
    gat = {key: gi for gi, (key, _) in enumerate(groups)}
    stages = {None: 4, "pro": 6, 1: len(groups)}
    oparts = list(zip((0,) + OSPLIT[:-1], OSPLIT))

    def kern(x_hbm, w_hbm, mean_hbm, var_hbm, g_hbm, b_hbm, o_hbm,
             xs, ws, wsu, lhs, ob, yb, pv, pb0, pb1, pb2, pb3,
             isem, osem, psem):
        pvb = (pb0, pb1, pb2, pb3)
        pcopies = [
            pltpu.make_async_copy(src, pvb[j], psem.at[0])
            for j, src in enumerate((mean_hbm, var_hbm, g_hbm, b_hbm))
        ]

        def params():
            for c in pcopies:
                c.wait()
            ld = lambda j: pvb[j][...].reshape(1, C).astype(f32)
            inv_std = r(1.0 / r(jnp.sqrt(r(ld(1) + 1e-5))))
            pv[0:1] = r(ld(2) * inv_std)
            pv[1:2] = ld(0)
            pv[2:3] = ld(3)

        def icopy(kind, i, gi):
            if kind == "x":
                bb, lo, hi = xch[i]
                return pltpu.make_async_copy(
                    x_hbm.at[bb, pl.ds(lo, hi - lo)],
                    xs.at[bb, pl.ds(H + lo, hi - lo)], isem.at[gi])
            if kind == "w":
                cs = pl.ds(i * TN, TN)
                return pltpu.make_async_copy(
                    w_hbm.at[:, cs], ws.at[:, cs], isem.at[gi])
            rs, cs = pl.ds(i * C, C), pl.ds(0, TN)
            return pltpu.make_async_copy(
                w_hbm.at[rs, cs], ws.at[rs, cs], isem.at[gi])

        gcopies = [[icopy(kind, i, gi) for kind, i in members]
                   for gi, (_, members) in enumerate(groups)]
        issued = [0]

        def issue_stage(key):
            if key in stages:
                for grp in gcopies[issued[0]:stages[key]]:
                    for c in grp:
                        c.start()
                issued[0] = stages[key]

        def gwait(key):
            if key not in gat:
                return
            gi = gat[key]
            assert gi < issued[0]
            for c in gcopies[gi]:
                c.wait()
            issue_stage(key)
            for kind, i in groups[gi][1]:
                if kind == "w":
                    cs = slice(i * TN, (i + 1) * TN)
                    wsu[:, cs] = pltpu.bitcast(ws[:, cs], u32)
                elif kind == "k":
                    wsu[i * C // 2:(i + 1) * C // 2, 0:TN] = pltpu.bitcast(
                        ws[i * C:(i + 1) * C, 0:TN], u32)

        def ocopy(t, n0, n1):
            i = t % nt
            r0 = i * TM if isinstance(t, int) else pl.multiple_of(i * TM, TM)
            cs = pl.ds(n0 * TN, (n1 - n0) * TN)
            return pltpu.make_async_copy(
                ob.at[t, :, cs], o_hbm.at[t // nt, pl.ds(r0, TM), cs],
                osem.at[0])

        def ostart(t, n):
            for n0, n1 in oparts:
                if n + 1 == n1:
                    ocopy(t, n0, n1).start()

        def build(bb, s0, slot, q0, nr, n):
            h = nr // 2
            c0, c1 = n * TN, (n + 1) * TN
            u = pltpu.bitcast(xs[bb, pl.ds(s0, nr + 2 * H), c0:c1], u32)
            lo = H // 2
            up, uc, un = u[lo - 1:lo - 1 + h], u[lo:lo + h], u[lo + 1:lo + 1 + h]
            lhs[slot, q0:q0 + h, c0:c1] = (up >> 16) | (uc << 16)
            lhs[slot, q0:q0 + h, C + c0:C + c1] = uc
            lhs[slot, q0:q0 + h, 2 * C + c0:2 * C + c1] = (uc >> 16) | (un << 16)

        def build_tile(t, n):
            if isinstance(t, int):
                build(t // nt, (t % nt) * TM, t % 2, 0, TM, n)
            else:
                tt = jnp.minimum(t, T - 1)
                build(tt // nt, pl.multiple_of((tt % nt) * TM, TM), t % 2, 0,
                      TM, n)

        def dots(t, y0, nr, n, before=None):
            cs = slice(n * TN, (n + 1) * TN)
            h, q0 = nr // 2, y0 // 2
            for k in range(K):
                if before is not None:
                    before(k)
                a_ = pltpu.bitcast(lhs[t % 2, q0:q0 + h, k * C:(k + 1) * C], bf)
                b_ = pltpu.bitcast(wsu[k * C // 2:(k + 1) * C // 2, cs], bf)
                p = r(jnp.dot(a_, b_, preferred_element_type=f32))
                if k == 0:
                    y = p
                elif k < K - 1:
                    y = r(y + p)
                else:
                    y = (y + p).astype(bf)
            yb[n % 2, y0:y0 + nr] = y

        def epilogue(t, n, lo, hi, npieces, chain):
            cs = slice(n * TN, (n + 1) * TN)
            rp = (hi - lo) // npieces
            for i in range(npieces):
                a, b_ = lo + i * rp, lo + (i + 1) * rp
                y = yb[n % 2, a:b_].astype(f32)
                if chain is not None and chain.get("prev") is not None:
                    never = jnp.broadcast_to(pv[3:4, 0:TN], y.shape) != 0
                    y = jnp.where(never, chain["prev"], y)
                y = r(r(r(y - pv[1:2, cs]) * pv[0:1, cs]) + pv[2:3, cs])
                d = r(1.0 + r(jnp.exp(-y)))
                sg = r(pl.reciprocal(d, approx=True))
                o = y * sg
                ob[t, a:b_, cs] = o.astype(bf)
                if chain is not None:
                    chain["prev"] = o

        for c in pcopies:
            c.start()
        issue_stage(None)
        zeros = jnp.zeros((H, C), bf)
        pv[3:4] = jnp.zeros((1, C), f32)
        for bb in range(B):
            xs[bb, 0:H] = zeros
            xs[bb, H + S:H + S + H] = zeros
        gwait("pro")
        for n in range(NN):
            build(0, 0, 0, 0, T1, n)

        units = [(c, n) for n in range(NN) for c in range(P)]
        chain = {}
        for j, (c, n) in enumerate(units):
            if j == 1:
                params()
            gwait(j)
            if n == 0 and c > 0:
                for n2 in range(NN):
                    build(0, c * T1, 0, c * T1 // 2, T1, n2)
            dots(0, c * T1, T1, n,
                 (lambda k: gwait(("k", k))) if j == 0 else None)
            if n > 0:
                epilogue(0, n - 1, c * T1, (c + 1) * T1, NPC, chain)
                if c == P - 1:
                    ostart(0, n - 1)
            b0, b1 = BUILD1
            for pc in range(NN):
                if b0 + (pc * (b1 - b0)) // NN == j:
                    build_tile(1, pc)

        def body(t, carry):
            @pl.when(t == REST_AT)
            def _():
                gwait("rest")

            chain = {}
            for n in range(NN):
                pt, pn = (t, n - 1) if n > 0 else (t - 1, NN - 1)
                dots(t, 0, TM, n)
                epilogue(pt, pn, 0, TM, NPC, chain)
                ostart(pt, pn)
                build_tile(t + 1, n)
            return carry

        jax.lax.fori_loop(1, T, body, 0)

        epilogue(T - 1, NN - 1, 0, TM, 1, None)
        ostart(T - 1, NN - 1)
        for t in range(T):
            for n0, n1 in oparts:
                ocopy(t, n0, n1).wait()

    return kern, T, len(groups)


@jax.jit
def pallas_standalone__batchnorm__prompt_kernel(
    x: jax.Array,
    w: jax.Array,
    mean: jax.Array,
    var: jax.Array,
    g: jax.Array,
    b: jax.Array,
):
    B, S, C = x.shape
    K = w.shape[0]
    bf = jnp.bfloat16
    kern, T, NG = _make_kernel(B, S, C, K)
    hbm = pl.BlockSpec(memory_space=pltpu.HBM)
    return pl.pallas_call(
        kern,
        in_specs=[hbm] * 6,
        out_specs=hbm,
        out_shape=jax.ShapeDtypeStruct((B, S, C), bf),
        scratch_shapes=[
            pltpu.VMEM((B, S + 2 * H, C), bf),
            pltpu.VMEM((K * C, C), bf),
            pltpu.VMEM((K * C // 2, C), jnp.uint32),
            pltpu.VMEM((2, TM // 2, K * C), jnp.uint32),
            pltpu.VMEM((T, TM, C), bf),
            pltpu.VMEM((2, TM, TN), bf),
            pltpu.VMEM((8, C), jnp.float32),
            pltpu.VMEM((C,), bf), pltpu.VMEM((C,), bf),
            pltpu.VMEM((C,), bf), pltpu.VMEM((C,), bf),
            pltpu.SemaphoreType.DMA((NG,)),
            pltpu.SemaphoreType.DMA((1,)),
            pltpu.SemaphoreType.DMA((1,)),
        ],
        compiler_params=pltpu.CompilerParams(vmem_limit_bytes=80 * 2**20),
    )(x, w.reshape(K * C, C), mean, var, g, b)
```

```python
import jax
import jax.numpy as jnp
from jax.experimental import pallas as pl
from jax.experimental.pallas import tpu as pltpu

TM = 512
T1 = 256
TN = 128
H = 16
NPC = 16
NPC1 = 8
OSPLIT = (4, 7, 8)
BUILD1 = (8, 16)
REST_AT = 2


def _make_kernel(B, S, C, K):
    nt = S // TM
    T = B * nt
    NN = C // TN
    P = TM // T1
    bf, f32, u32 = jnp.bfloat16, jnp.float32, jnp.uint32
    r = lambda a: a.astype(bf).astype(f32)

    xch = [(0, 0 if c == 0 else c * T1 + H, (c + 1) * T1 + H) for c in range(P)]
    for t in range(1, T):
        i = t % nt
        xch.append((t // nt, 0 if i == 0 else i * TM + H,
                    min(S, (i + 1) * TM + H)))

    groups = [
        ("pro", [("x", 0)]),
        (("k", 0), [("k", 0)]),
        (("k", 1), [("k", 1)]),
        (("k", 2), [("k", 2)]),
        (1, [("x", 1)]),
        (2, [("w", 1)]),
        (4, [("w", 2), ("w", 3)]),
        (8, [("x", 2), ("w", 4), ("w", 5)]),
        (12, [("w", 6), ("w", 7), ("x", 3)]),
        ("rest", [("x", c) for c in range(4, len(xch))]),
    ]
    gat = {key: gi for gi, (key, _) in enumerate(groups)}
    stages = {None: 4, "pro": 6, 1: len(groups)}
    oparts = list(zip((0,) + OSPLIT[:-1], OSPLIT))

    def kern(x_hbm, w_hbm, mean_hbm, var_hbm, g_hbm, b_hbm, o_hbm,
             xs, ws, wsu, lhs, ob, yb, pv, pb0, pb1, pb2, pb3,
             isem, osem, psem):
        pvb = (pb0, pb1, pb2, pb3)
        pcopies = [
            pltpu.make_async_copy(src, pvb[j], psem.at[0])
            for j, src in enumerate((mean_hbm, var_hbm, g_hbm, b_hbm))
        ]

        def params():
            for c in pcopies:
                c.wait()
            ld = lambda j: pvb[j][...].reshape(1, C).astype(f32)
            inv_std = r(1.0 / r(jnp.sqrt(r(ld(1) + 1e-5))))
            pv[0:1] = r(ld(2) * inv_std)
            pv[1:2] = ld(0)
            pv[2:3] = ld(3)

        def icopy(kind, i, gi):
            if kind == "x":
                bb, lo, hi = xch[i]
                return pltpu.make_async_copy(
                    x_hbm.at[bb, pl.ds(lo, hi - lo)],
                    xs.at[bb, pl.ds(H + lo, hi - lo)], isem.at[gi])
            if kind == "w":
                cs = pl.ds(i * TN, TN)
                return pltpu.make_async_copy(
                    w_hbm.at[:, cs], ws.at[:, cs], isem.at[gi])
            rs, cs = pl.ds(i * C, C), pl.ds(0, TN)
            return pltpu.make_async_copy(
                w_hbm.at[rs, cs], ws.at[rs, cs], isem.at[gi])

        gcopies = [[icopy(kind, i, gi) for kind, i in members]
                   for gi, (_, members) in enumerate(groups)]
        issued = [0]

        def issue_stage(key):
            if key in stages:
                for grp in gcopies[issued[0]:stages[key]]:
                    for c in grp:
                        c.start()
                issued[0] = stages[key]

        def gwait(key):
            if key not in gat:
                return
            gi = gat[key]
            assert gi < issued[0]
            for c in gcopies[gi]:
                c.wait()
            issue_stage(key)
            for kind, i in groups[gi][1]:
                if kind == "w":
                    cs = slice(i * TN, (i + 1) * TN)
                    wsu[:, cs] = pltpu.bitcast(ws[:, cs], u32)
                elif kind == "k":
                    wsu[i * C // 2:(i + 1) * C // 2, 0:TN] = pltpu.bitcast(
                        ws[i * C:(i + 1) * C, 0:TN], u32)

        def ocopy(t, n0, n1):
            i = t % nt
            r0 = i * TM if isinstance(t, int) else pl.multiple_of(i * TM, TM)
            cs = pl.ds(n0 * TN, (n1 - n0) * TN)
            return pltpu.make_async_copy(
                ob.at[t, :, cs], o_hbm.at[t // nt, pl.ds(r0, TM), cs],
                osem.at[0])

        def ostart(t, n):
            for n0, n1 in oparts:
                if n + 1 == n1:
                    ocopy(t, n0, n1).start()

        def build(bb, s0, slot, q0, nr, n):
            h = nr // 2
            c0, c1 = n * TN, (n + 1) * TN
            u = pltpu.bitcast(xs[bb, pl.ds(s0, nr + 2 * H), c0:c1], u32)
            lo = H // 2
            up, uc, un = u[lo - 1:lo - 1 + h], u[lo:lo + h], u[lo + 1:lo + 1 + h]
            lhs[slot, q0:q0 + h, c0:c1] = (up >> 16) | (uc << 16)
            lhs[slot, q0:q0 + h, C + c0:C + c1] = uc
            lhs[slot, q0:q0 + h, 2 * C + c0:2 * C + c1] = (uc >> 16) | (un << 16)

        def build_tile(t, n):
            if isinstance(t, int):
                build(t // nt, (t % nt) * TM, t % 2, 0, TM, n)
            else:
                tt = jnp.minimum(t, T - 1)
                build(tt // nt, pl.multiple_of((tt % nt) * TM, TM), t % 2, 0,
                      TM, n)

        def dots(t, y0, nr, n, before=None):
            cs = slice(n * TN, (n + 1) * TN)
            h, q0 = nr // 2, y0 // 2
            for k in range(K):
                if before is not None:
                    before(k)
                a_ = pltpu.bitcast(lhs[t % 2, q0:q0 + h, k * C:(k + 1) * C], bf)
                b_ = pltpu.bitcast(wsu[k * C // 2:(k + 1) * C // 2, cs], bf)
                p = r(jnp.dot(a_, b_, preferred_element_type=f32))
                if k == 0:
                    y = p
                elif k < K - 1:
                    y = r(y + p)
                else:
                    y = (y + p).astype(bf)
            yb[n % 2, y0:y0 + nr] = y

        def epilogue(t, n, lo, hi, npieces, chain):
            cs = slice(n * TN, (n + 1) * TN)
            rp = (hi - lo) // npieces
            for i in range(npieces):
                a, b_ = lo + i * rp, lo + (i + 1) * rp
                y = yb[n % 2, a:b_].astype(f32)
                if chain is not None and chain.get("prev") is not None:
                    never = jnp.broadcast_to(pv[3:4, 0:TN], y.shape) != 0
                    y = jnp.where(never, chain["prev"], y)
                y = r(r(r(y - pv[1:2, cs]) * pv[0:1, cs]) + pv[2:3, cs])
                d = r(1.0 + r(jnp.exp(-y)))
                sg = r(1.0 / d)
                o = y * sg
                ob[t, a:b_, cs] = o.astype(bf)
                if chain is not None:
                    chain["prev"] = o

        for c in pcopies:
            c.start()
        issue_stage(None)
        zeros = jnp.zeros((H, C), bf)
        pv[3:4] = jnp.zeros((1, C), f32)
        for bb in range(B):
            xs[bb, 0:H] = zeros
            xs[bb, H + S:H + S + H] = zeros
        gwait("pro")
        for n in range(NN):
            build(0, 0, 0, 0, T1, n)

        units = [(c, n) for n in range(NN) for c in range(P)]
        chain = {}
        for j, (c, n) in enumerate(units):
            if j == 1:
                params()
            gwait(j)
            if n == 0 and c > 0:
                for n2 in range(NN):
                    build(0, c * T1, 0, c * T1 // 2, T1, n2)
            dots(0, c * T1, T1, n,
                 (lambda k: gwait(("k", k))) if j == 0 else None)
            if n > 0:
                epilogue(0, n - 1, c * T1, (c + 1) * T1, NPC1, chain)
                if c == P - 1:
                    ostart(0, n - 1)
            b0, b1 = BUILD1
            for pc in range(NN):
                if b0 + (pc * (b1 - b0)) // NN == j:
                    build_tile(1, pc)

        def body(t, carry):
            @pl.when(t == REST_AT)
            def _():
                gwait("rest")

            chain = {}
            for n in range(NN):
                pt, pn = (t, n - 1) if n > 0 else (t - 1, NN - 1)
                dots(t, 0, TM, n)
                epilogue(pt, pn, 0, TM, NPC, chain)
                ostart(pt, pn)
                build_tile(t + 1, n)
            return carry

        jax.lax.fori_loop(1, T, body, 0)

        epilogue(T - 1, NN - 1, 0, TM, 1, None)
        ostart(T - 1, NN - 1)
        for t in range(T):
            for n0, n1 in oparts:
                ocopy(t, n0, n1).wait()

    return kern, T, len(groups)


@jax.jit
def pallas_standalone__batchnorm__prompt_kernel(
    x: jax.Array,
    w: jax.Array,
    mean: jax.Array,
    var: jax.Array,
    g: jax.Array,
    b: jax.Array,
):
    B, S, C = x.shape
    K = w.shape[0]
    bf = jnp.bfloat16
    kern, T, NG = _make_kernel(B, S, C, K)
    hbm = pl.BlockSpec(memory_space=pltpu.HBM)
    return pl.pallas_call(
        kern,
        in_specs=[hbm] * 6,
        out_specs=hbm,
        out_shape=jax.ShapeDtypeStruct((B, S, C), bf),
        scratch_shapes=[
            pltpu.VMEM((B, S + 2 * H, C), bf),
            pltpu.VMEM((K * C, C), bf),
            pltpu.VMEM((K * C // 2, C), jnp.uint32),
            pltpu.VMEM((2, TM // 2, K * C), jnp.uint32),
            pltpu.VMEM((T, TM, C), bf),
            pltpu.VMEM((2, TM, TN), bf),
            pltpu.VMEM((8, C), jnp.float32),
            pltpu.VMEM((C,), bf), pltpu.VMEM((C,), bf),
            pltpu.VMEM((C,), bf), pltpu.VMEM((C,), bf),
            pltpu.SemaphoreType.DMA((NG,)),
            pltpu.SemaphoreType.DMA((1,)),
            pltpu.SemaphoreType.DMA((1,)),
        ],
        compiler_params=pltpu.CompilerParams(vmem_limit_bytes=80 * 2**20),
    )(x, w.reshape(K * C, C), mean, var, g, b)
```

```python
import jax
import jax.numpy as jnp
from jax.experimental import pallas as pl
from jax.experimental.pallas import tpu as pltpu

TM = 512
T1 = 256
TN = 128
H = 16
NPC = 16
NPC1 = 8
OSPLIT = (4, 7, 8)
NSPLIT = 2
BUILD1 = (6, 10)
REST_AT = 2


def _make_kernel(B, S, C, K):
    nt = S // TM
    T = B * nt
    NN = C // TN
    P = TM // T1
    bf, f32, u32 = jnp.bfloat16, jnp.float32, jnp.uint32
    r = lambda a: a.astype(bf).astype(f32)

    xch = [(0, 0 if c == 0 else c * T1 + H, (c + 1) * T1 + H) for c in range(P)]
    for t in range(1, T):
        i = t % nt
        xch.append((t // nt, 0 if i == 0 else i * TM + H,
                    min(S, (i + 1) * TM + H)))

    groups = [
        ("pro", [("x", 0)]),
        (("k", 0), [("k", 0)]),
        (("k", 1), [("k", 1)]),
        (("k", 2), [("k", 2)]),
        (1, [("x", 1)]),
        (2, [("w", 1)]),
        (4, [("w", 2), ("w", 3)]),
        (6, [("x", 2), ("w", 4), ("w", 5)]),
        (8, [("w", 6), ("w", 7), ("x", 3)]),
        ("rest", [("x", c) for c in range(4, len(xch))]),
    ]
    gat = {key: gi for gi, (key, _) in enumerate(groups)}
    stages = {None: 4, "pro": 6, 1: len(groups)}
    oparts = list(zip((0,) + OSPLIT[:-1], OSPLIT))

    def kern(x_hbm, w_hbm, mean_hbm, var_hbm, g_hbm, b_hbm, o_hbm,
             xs, ws, wsu, lhs, ob, yb, pv, pb0, pb1, pb2, pb3,
             isem, osem, psem):
        pvb = (pb0, pb1, pb2, pb3)
        pcopies = [
            pltpu.make_async_copy(src, pvb[j], psem.at[0])
            for j, src in enumerate((mean_hbm, var_hbm, g_hbm, b_hbm))
        ]

        def params():
            for c in pcopies:
                c.wait()
            ld = lambda j: pvb[j][...].reshape(1, C).astype(f32)
            inv_std = r(1.0 / r(jnp.sqrt(r(ld(1) + 1e-5))))
            pv[0:1] = r(ld(2) * inv_std)
            pv[1:2] = ld(0)
            pv[2:3] = ld(3)

        def icopy(kind, i, gi):
            if kind == "x":
                bb, lo, hi = xch[i]
                return pltpu.make_async_copy(
                    x_hbm.at[bb, pl.ds(lo, hi - lo)],
                    xs.at[bb, pl.ds(H + lo, hi - lo)], isem.at[gi])
            if kind == "w":
                cs = pl.ds(i * TN, TN)
                return pltpu.make_async_copy(
                    w_hbm.at[:, cs], ws.at[:, cs], isem.at[gi])
            rs, cs = pl.ds(i * C, C), pl.ds(0, TN)
            return pltpu.make_async_copy(
                w_hbm.at[rs, cs], ws.at[rs, cs], isem.at[gi])

        gcopies = [[icopy(kind, i, gi) for kind, i in members]
                   for gi, (_, members) in enumerate(groups)]
        issued = [0]

        def issue_stage(key):
            if key in stages:
                for grp in gcopies[issued[0]:stages[key]]:
                    for c in grp:
                        c.start()
                issued[0] = stages[key]

        def gwait(key):
            if key not in gat:
                return
            gi = gat[key]
            assert gi < issued[0]
            for c in gcopies[gi]:
                c.wait()
            issue_stage(key)
            for kind, i in groups[gi][1]:
                if kind == "w":
                    cs = slice(i * TN, (i + 1) * TN)
                    wsu[:, cs] = pltpu.bitcast(ws[:, cs], u32)
                elif kind == "k":
                    wsu[i * C // 2:(i + 1) * C // 2, 0:TN] = pltpu.bitcast(
                        ws[i * C:(i + 1) * C, 0:TN], u32)

        def ocopy(t, n0, n1):
            i = t % nt
            r0 = i * TM if isinstance(t, int) else pl.multiple_of(i * TM, TM)
            cs = pl.ds(n0 * TN, (n1 - n0) * TN)
            return pltpu.make_async_copy(
                ob.at[t, :, cs], o_hbm.at[t // nt, pl.ds(r0, TM), cs],
                osem.at[0])

        def ostart(t, n):
            for n0, n1 in oparts:
                if n + 1 == n1:
                    ocopy(t, n0, n1).start()

        def build(bb, s0, slot, q0, nr, n):
            h = nr // 2
            c0, c1 = n * TN, (n + 1) * TN
            u = pltpu.bitcast(xs[bb, pl.ds(s0, nr + 2 * H), c0:c1], u32)
            lo = H // 2
            up, uc, un = u[lo - 1:lo - 1 + h], u[lo:lo + h], u[lo + 1:lo + 1 + h]
            lhs[slot, q0:q0 + h, c0:c1] = (up >> 16) | (uc << 16)
            lhs[slot, q0:q0 + h, C + c0:C + c1] = uc
            lhs[slot, q0:q0 + h, 2 * C + c0:2 * C + c1] = (uc >> 16) | (un << 16)

        def build_tile(t, n):
            if isinstance(t, int):
                build(t // nt, (t % nt) * TM, t % 2, 0, TM, n)
            else:
                tt = jnp.minimum(t, T - 1)
                build(tt // nt, pl.multiple_of((tt % nt) * TM, TM), t % 2, 0,
                      TM, n)

        def dots(t, y0, nr, n, before=None):
            cs = slice(n * TN, (n + 1) * TN)
            h, q0 = nr // 2, y0 // 2
            for k in range(K):
                if before is not None:
                    before(k)
                a_ = pltpu.bitcast(lhs[t % 2, q0:q0 + h, k * C:(k + 1) * C], bf)
                b_ = pltpu.bitcast(wsu[k * C // 2:(k + 1) * C // 2, cs], bf)
                p = r(jnp.dot(a_, b_, preferred_element_type=f32))
                if k == 0:
                    y = p
                elif k < K - 1:
                    y = r(y + p)
                else:
                    y = (y + p).astype(bf)
            yb[n % 2, y0:y0 + nr] = y

        def epilogue(t, n, lo, hi, npieces, chain):
            cs = slice(n * TN, (n + 1) * TN)
            rp = (hi - lo) // npieces
            for i in range(npieces):
                a, b_ = lo + i * rp, lo + (i + 1) * rp
                y = yb[n % 2, a:b_].astype(f32)
                if chain is not None and chain.get("prev") is not None:
                    never = jnp.broadcast_to(pv[3:4, 0:TN], y.shape) != 0
                    y = jnp.where(never, chain["prev"], y)
                y = r(r(r(y - pv[1:2, cs]) * pv[0:1, cs]) + pv[2:3, cs])
                d = r(1.0 + r(jnp.exp(-y)))
                sg = r(1.0 / d)
                o = y * sg
                ob[t, a:b_, cs] = o.astype(bf)
                if chain is not None:
                    chain["prev"] = o

        for c in pcopies:
            c.start()
        issue_stage(None)
        zeros = jnp.zeros((H, C), bf)
        pv[3:4] = jnp.zeros((1, C), f32)
        for bb in range(B):
            xs[bb, 0:H] = zeros
            xs[bb, H + S:H + S + H] = zeros
        gwait("pro")
        for n in range(NN):
            build(0, 0, 0, 0, T1, n)

        units = []
        for n in range(NN):
            if n < NSPLIT:
                units += [(c * T1, T1, n) for c in range(P)]
            else:
                units += [(0, TM, n)]
        chain = {}
        for j, (y0, nr, n) in enumerate(units):
            if j == 1:
                params()
            gwait(j)
            if n == 0 and y0 > 0:
                for n2 in range(NN):
                    build(0, y0, 0, y0 // 2, T1, n2)
            dots(0, y0, nr, n,
                 (lambda k: gwait(("k", k))) if j == 0 else None)
            if n > 0:
                epilogue(0, n - 1, y0, y0 + nr, NPC1 * (nr // T1), chain)
                if y0 + nr == TM:
                    ostart(0, n - 1)
            b0, b1 = BUILD1
            for pc in range(NN):
                if b0 + (pc * (b1 - b0)) // NN == j:
                    build_tile(1, pc)

        def body(t, carry):
            @pl.when(t == REST_AT)
            def _():
                gwait("rest")

            chain = {}
            for n in range(NN):
                pt, pn = (t, n - 1) if n > 0 else (t - 1, NN - 1)
                dots(t, 0, TM, n)
                epilogue(pt, pn, 0, TM, NPC, chain)
                ostart(pt, pn)
                build_tile(t + 1, n)
            return carry

        jax.lax.fori_loop(1, T, body, 0)

        epilogue(T - 1, NN - 1, 0, TM, 1, None)
        ostart(T - 1, NN - 1)
        for t in range(T):
            for n0, n1 in oparts:
                ocopy(t, n0, n1).wait()

    return kern, T, len(groups)


@jax.jit
def pallas_standalone__batchnorm__prompt_kernel(
    x: jax.Array,
    w: jax.Array,
    mean: jax.Array,
    var: jax.Array,
    g: jax.Array,
    b: jax.Array,
):
    B, S, C = x.shape
    K = w.shape[0]
    bf = jnp.bfloat16
    kern, T, NG = _make_kernel(B, S, C, K)
    hbm = pl.BlockSpec(memory_space=pltpu.HBM)
    return pl.pallas_call(
        kern,
        in_specs=[hbm] * 6,
        out_specs=hbm,
        out_shape=jax.ShapeDtypeStruct((B, S, C), bf),
        scratch_shapes=[
            pltpu.VMEM((B, S + 2 * H, C), bf),
            pltpu.VMEM((K * C, C), bf),
            pltpu.VMEM((K * C // 2, C), jnp.uint32),
            pltpu.VMEM((2, TM // 2, K * C), jnp.uint32),
            pltpu.VMEM((T, TM, C), bf),
            pltpu.VMEM((2, TM, TN), bf),
            pltpu.VMEM((8, C), jnp.float32),
            pltpu.VMEM((C,), bf), pltpu.VMEM((C,), bf),
            pltpu.VMEM((C,), bf), pltpu.VMEM((C,), bf),
            pltpu.SemaphoreType.DMA((NG,)),
            pltpu.SemaphoreType.DMA((1,)),
            pltpu.SemaphoreType.DMA((1,)),
        ],
        compiler_params=pltpu.CompilerParams(vmem_limit_bytes=80 * 2**20),
    )(x, w.reshape(K * C, C), mean, var, g, b)
```
